```python
import os as _os
_os.environ.setdefault("JAX_PLATFORMS", "cpu")
import jax
import jax.numpy as jnp

def _softmax(x, axis=-1):
    return jax.nn.softmax(x, axis=axis)
def _gelu(x):
    return jax.nn.gelu(x, approximate=True)
def _silu(x):
    return jax.nn.silu(x)
def _sigmoid(x):
    return jax.nn.sigmoid(x)
def _layernorm(x, axis=-1, eps=1e-5):
    m = jnp.mean(x, axis=axis, keepdims=True)
    v = jnp.var(x, axis=axis, keepdims=True)
    return (x - m) / jnp.sqrt(v + eps)
def _scatter_add(tgt, idx, src, axis=0):
    return tgt.at[idx].add(src)
def _segment_sum(src, seg, n):
    return jax.ops.segment_sum(src, seg, n)
class _Rng:
    def __init__(self, key):
        self._k = key
    def _next(self):
        self._k, sub = jax.random.split(self._k)
        return sub
    def normal(self, shape):
        return jax.random.normal(self._next(), shape, dtype=jnp.bfloat16)
    def randint(self, lo, hi, shape):
        return jax.random.randint(self._next(), shape, lo, hi, dtype=jnp.int32)
    def uniform(self, shape, lo=0.0, hi=1.0):
        return jax.random.uniform(self._next(), shape, jnp.bfloat16, lo, hi)
    def permutation(self, n):
        return jax.random.permutation(self._next(), n)


kernel_name = 'standalone__seq2seq_rnn_t_joint__speech'

def setup_inputs():
    _rng = _Rng(jax.random.key(int.from_bytes(__import__("os").urandom(4), "little")))
    _w = (lambda a: (lambda t: t.astype(jnp.bfloat16) if jnp.issubdtype(t.dtype, jnp.floating) else t)(jnp.asarray(a)))
    B, T, D, K = 2, 16000, 256, 31
    U = 8
    sc = (1.0 / (K * D)) ** 0.5
    sd = (1.0 / D) ** 0.5
    return {
        "x": _w((lambda *s: _rng.normal(s) * 0.2)(B, T, D) * 0.5),
        "w1": _w((lambda *s: _rng.normal(s) * 1.6)(K, D, D) * sc),
        "w2": _w((lambda *s: _rng.normal(s) * 1.6)(K, D, D) * sc),
        "g": _w((lambda *s: _rng.normal(s) * 1.6)(B, U, D) * 0.5),
        "w_f": _w((lambda *s: _rng.normal(s) * 1.6)(D, D) * sd),
        "w_g": _w((lambda *s: _rng.normal(s) * 1.6)(D, D) * sd),
        "w_o": _w((lambda *s: _rng.normal(s) * 1.6)(D, D) * sd),
    }

def reference(x, w1, w2, g, w_f, w_g, w_o):
    B, T, D = x.shape
    K = w1.shape[0]
    pad = K // 2
    xp = jnp.pad(x, ((0,0),(pad,pad),(0,0)))
    h = jnp.zeros_like(x)
    for i in range(K):
        h = h + jnp.einsum("btc,cd->btd", xp[:, i:i+T, :], w1[i])
    h = _gelu(h)[:, ::2, :]
    T1 = h.shape[1]
    hp = jnp.pad(h, ((0,0),(pad,pad),(0,0)))
    f = jnp.zeros_like(h)
    for i in range(K):
        f = f + jnp.einsum("btc,cd->btd", hp[:, i:i+T1, :], w2[i])
    f = _gelu(f)[:, ::2, :]
    fe = jnp.einsum("btd,de->bte", f, w_f)
    ge = jnp.einsum("bud,de->bue", g, w_g)
    j = jnp.tanh(fe[:, :, None, :] + ge[:, None, :, :])
    return jnp.einsum("btud,dv->btuv", j, w_o)
```

```python
import math

import jax
import jax.numpy as jnp
import jax.experimental.pallas as pl
import jax.experimental.pallas.tpu as pltpu
from jax import lax

N = 32
TAPS = 16
L = N - TAPS + 1
NC = 3 * (N // 2 - 1) + 2
MC = 240
LANE = 128
JT = 400


def _neg(a):
    return None if a is None else (-a[0], a[1])


def _add(a, b):
    if a is None:
        return b
    if b is None:
        return a
    if a[0] == b[0]:
        return (a[0], a[1] + b[1])
    return (1, a[1] - b[1]) if a[0] > 0 else (1, b[1] - a[1])


def _sub(a, b):
    return _add(a, _neg(b))


def _mul(a, c):
    if a is None or abs(c) < 1e-12:
        return None
    if abs(abs(c) - 1.0) < 1e-12:
        return a if c > 0 else _neg(a)
    return (1, a[1] * (c * a[0]))


def _val(a):
    return a[1] if a[0] > 0 else -a[1]


def _twiddle(re, im, c, s):
    if re is not None and im is not None and abs(abs(c) - abs(s)) < 1e-12:
        sg = 1.0 if c * s > 0 else -1.0
        return (_mul(_sub(re, _mul(im, sg)), c), _mul(_add(im, _mul(re, sg)), c))
    return (_sub(_mul(re, c), _mul(im, s)), _add(_mul(re, s), _mul(im, c)))


def _rfft(x):
    n = len(x)
    if n == 1:
        return [(x[0], None)]
    if n == 2:
        return [(_add(x[0], x[1]), None), (_sub(x[0], x[1]), None)]
    e, o = _rfft(x[0::2]), _rfft(x[1::2])
    h, q = n // 2, n // 4
    out = [None] * (h + 1)
    out[0] = (_add(e[0][0], o[0][0]), None)
    out[h] = (_sub(e[0][0], o[0][0]), None)
    out[q] = (e[q][0], _neg(o[q][0]))
    for k in range(1, q):
        a = 2 * math.pi * k / n
        tr, ti = _twiddle(o[k][0], o[k][1], math.cos(a), -math.sin(a))
        out[k] = (_add(e[k][0], tr), _add(e[k][1], ti))
        out[h - k] = (_sub(e[k][0], tr), _sub(ti, e[k][1]))
    return out


def _irfft(X, need):
    h = len(X) - 1
    n = 2 * h
    if n == 2:
        return {i: (_add if i == 0 else _sub)(X[0][0], X[1][0]) for i in need}
    q = n // 4
    ne = sorted(i // 2 for i in need if i % 2 == 0)
    no = sorted(i // 2 for i in need if i % 2 == 1)
    out = {}
    if ne:
        e = [None] * (q + 1)
        e[0] = (_add(X[0][0], X[h][0]), None)
        e[q] = (X[q][0], None)
        for k in range(1, q):
            e[k] = (_add(X[k][0], X[h - k][0]), _sub(X[k][1], X[h - k][1]))
        out.update({2 * i: v for i, v in _irfft(e, ne).items()})
    if no:
        o = [None] * (q + 1)
        o[0] = (_sub(X[0][0], X[h][0]), None)
        o[q] = (_neg(X[q][1]), None)
        for k in range(1, q):
            a = 2 * math.pi * k / n
            o[k] = _twiddle(_sub(X[k][0], X[h - k][0]), _add(X[k][1], X[h - k][1]),
                            math.cos(a), math.sin(a))
        out.update({2 * i + 1: v for i, v in _irfft(o, no).items()})
    return out


def _data_components(x):
    X = _rfft(x)
    out = [X[0][0], X[N // 2][0]]
    for k in range(1, N // 2):
        out += [_add(X[k][0], X[k][1]), X[k][1], X[k][0]]
    return out


def _weight_components(w):
    W = _rfft(w)
    out = [W[0][0], W[N // 2][0]]
    for k in range(1, N // 2):
        vr, vi = _add(W[k][0], W[k][0]), _neg(_add(W[k][1], W[k][1]))
        out += [vr, _neg(_add(vr, vi)), _sub(vi, vr)]
    return out


def _gelu(x):
    c = math.sqrt(2.0 / math.pi)
    return (0.5 * x) * (1.0 + jnp.tanh(x * (c + (c * 0.044715) * (x * x))))


def _kernel(x_hbm, w1_hbm, w2_hbm, g_ref, wf_ref, wg_ref, wo_ref, out_ref,
            xs, wraw, wh1, wh2, xh, yh, hs, fb, fes, sems, *, T, K, D, U):
    b, s = pl.program_id(0), pl.program_id(1)
    T1, T2 = T // 2, T // 4
    NCOL = D // LANE
    f32, bf16 = jnp.float32, jnp.bfloat16

    def x_copy(bb, c):
        return pltpu.make_async_copy(x_hbm.at[bb, :, pl.ds(c * LANE, LANE)],
                                     xs.bitcast(bf16).at[c, pl.ds(TAPS, T), :], sems.at[c])

    def transform_weights(wh):
        def body(i, _):
            r = pl.multiple_of((i // NCOL) * 16, 16)
            c = pl.multiple_of((i % NCOL) * LANE, LANE)
            for ph in range(2):
                taps = []
                for m in range(N):
                    k = 2 * m - 1 + ph
                    ok = m < TAPS and 0 <= k < K
                    taps.append((1, wraw[k, pl.ds(r, 16), pl.ds(c, LANE)].astype(f32) * (1.0 / N))
                                if ok else None)
                for j, v in enumerate(_weight_components(taps)):
                    wh[j, pl.ds(ph * D + r, 16), pl.ds(c, LANE)] = _val(v).astype(bf16)
        lax.fori_loop(0, (D // 16) * NCOL, body, None)

    def forward(load, b0):
        def body(i, _):
            r = pl.multiple_of(i * 8, 8)
            for c in range(NCOL):
                for ph, sig in enumerate(load(b0 + r, c)):
                    for j, v in enumerate(_data_components([(1, t) for t in sig])):
                        xh[j, pl.ds(r, 8), pl.ds(ph * D + c * LANE, LANE)] = _val(v).astype(bf16)
        lax.fori_loop(0, MC // 8, body, None)

    def spectral(wh):
        dot = lambda j: jnp.dot(xh[j], wh[j], preferred_element_type=f32)
        yh[0] = dot(0)
        yh[1] = dot(1)

        def body(k, _):
            k1 = dot(3 * k + 2)
            yh[2 * k + 2] = k1 + dot(3 * k + 3)
            yh[2 * k + 3] = k1 + dot(3 * k + 4)
        lax.fori_loop(0, N // 2 - 1, body, None)

    def inverse(emit):
        def body(i, _):
            r = pl.multiple_of(i * 8, 8)
            for c in range(NCOL):
                ld = lambda j: (1, yh[j, pl.ds(r, 8), pl.ds(c * LANE, LANE)])
                X = [(ld(0), None)] + [(ld(2 * k), ld(2 * k + 1)) for k in range(1, N // 2)]
                X.append((ld(1), None))
                y = _irfft(X, list(range(L)))
                for n in range(L):
                    emit(r, c, n, _gelu(_val(y[n])))
        lax.fori_loop(0, MC // 8, body, None)

    def load_x(blk, c):
        w = [xs[c, pl.ds(blk * L + m, 8, stride=L), :] for m in range(N)]
        yield [pltpu.bitcast(t << 16, f32) for t in w]
        yield [pltpu.bitcast(t & jnp.uint32(0xFFFF0000), f32) for t in w]

    def load_h(blk, c):
        for ph in range(2):
            yield [hs[c, pl.ds(blk * 2 * L + 2 * m + ph, 8, stride=2 * L), :] for m in range(N)]

    @pl.when(jnp.logical_and(b == 0, s == 0))
    def _():
        cw = pltpu.make_async_copy(w1_hbm, wraw, sems.at[NCOL])
        cw.start()
        for c in range(NCOL):
            x_copy(0, c).start()
            xs[c, pl.ds(0, TAPS // 2), :] = jnp.zeros((TAPS // 2, LANE), jnp.uint32)
            tail = xs.shape[1] - TAPS // 2 - T1
            xs[c, pl.ds(TAPS // 2 + T1, tail), :] = jnp.zeros((tail, LANE), jnp.uint32)
            hs[c, pl.ds(0, TAPS), :] = jnp.zeros((TAPS, LANE), f32)
            done = TAPS + 2 * MC * L
            hs[c, pl.ds(done, hs.shape[1] - done), :] = jnp.zeros((hs.shape[1] - done, LANE), f32)
        cw.wait()
        with jax.named_scope("wt"):
            transform_weights(wh1)
        cw = pltpu.make_async_copy(w2_hbm, wraw, sems.at[NCOL])
        cw.start()
        cw.wait()
        transform_weights(wh2)

    @pl.when(s == 0)
    def _():
        for c in range(NCOL):
            x_copy(b, c).wait()

        def conv1_chunk(i, _):
            b0 = i * MC

            def emit(r, c, n, v):
                p0 = (b0 + r) * L + n
                pos = p0 + L * lax.broadcasted_iota(jnp.int32, (8, LANE), 0)
                hs[c, pl.ds(TAPS + p0, 8, stride=L), :] = jnp.where(pos < T1, v, 0.0)
            with jax.named_scope("f1"):
                forward(load_x, b0)
            with jax.named_scope("s1"):
                spectral(wh1)
            with jax.named_scope("i1"):
                inverse(emit)
        lax.fori_loop(0, 2, conv1_chunk, None)

        @pl.when(b + 1 < pl.num_programs(0))
        def _():
            for c in range(NCOL):
                x_copy(b + 1, c).start()

        def emit2(r, c, n, v):
            fb[n, pl.ds(r, 8), pl.ds(c * LANE, LANE)] = v.astype(bf16)
        with jax.named_scope("f2"):
            forward(load_h, 0)
        with jax.named_scope("s2"):
            spectral(wh2)
        with jax.named_scope("i2"):
            inverse(emit2)

        def fe_body(n, _):
            fe = jnp.dot(fb[n], wf_ref[...], preferred_element_type=f32)
            for c in range(NCOL):
                fes[c, pl.ds(n, MC, stride=L), :] = fe[:, c * LANE:(c + 1) * LANE]
        with jax.named_scope("fe"):
            lax.fori_loop(0, L, fe_body, None)

    ge = jnp.dot(g_ref[0], wg_ref[...], preferred_element_type=f32)
    G = 40

    def joint(i, _):
        t0 = s * JT + i * G
        rows = []
        for t in range(G):
            fe = jnp.concatenate([fes[c, pl.ds(t0 + t, 1), :] for c in range(NCOL)], axis=1)
            rows.append(jnp.tanh(fe + ge))
        j = jnp.concatenate(rows, axis=0).astype(bf16)
        o = jnp.dot(j, wo_ref[...], preferred_element_type=f32)
        out_ref[0, pl.ds(pl.multiple_of(i * G * U, G * U), G * U), :] = o.astype(bf16)
    with jax.named_scope("joint"):
        lax.fori_loop(0, JT // G, joint, None)


@jax.jit
def pallas_standalone__seq2seq_rnn_t_joint__speech_kernel(x, w1, w2, g, w_f, w_g, w_o):
    B, T, D = x.shape
    K, U = w1.shape[0], g.shape[1]
    T2 = T // 4
    assert K == 2 * TAPS - 1 and T % 4 == 0 and T2 % JT == 0 and U == 8
    assert 2 * MC * L >= T // 2 and MC * L >= T2
    ncol = D // LANE
    rows = lambda n: -(-(2 * ((n - 1) * L + N)) // 16) * 16
    full = lambda a: pl.BlockSpec(a.shape, lambda b, s: (0,) * a.ndim)
    hbm = pl.BlockSpec(memory_space=pl.ANY)
    kern = lambda *refs: _kernel(*refs, T=T, K=K, D=D, U=U)
    out = pl.pallas_call(
        kern,
        grid=(B, T2 // JT),
        in_specs=[hbm, hbm, hbm, pl.BlockSpec((1, U, D), lambda b, s: (b, 0, 0)),
                  full(w_f), full(w_g), full(w_o)],
        out_specs=pl.BlockSpec((1, JT * U, w_o.shape[1]), lambda b, s: (b, s, 0)),
        out_shape=jax.ShapeDtypeStruct((B, T2 * U, w_o.shape[1]), x.dtype),
        scratch_shapes=[
            pltpu.VMEM((ncol, rows(2 * MC) // 2, LANE), jnp.uint32),
            pltpu.VMEM((K, D, D), jnp.bfloat16),
            pltpu.VMEM((NC, 2 * D, D), jnp.bfloat16),
            pltpu.VMEM((NC, 2 * D, D), jnp.bfloat16),
            pltpu.VMEM((NC, MC, 2 * D), jnp.bfloat16),
            pltpu.VMEM((N, MC, D), jnp.float32),
            pltpu.VMEM((ncol, max(rows(MC), TAPS + 2 * MC * L + 8), LANE), jnp.float32),
            pltpu.VMEM((L, MC, D), jnp.bfloat16),
            pltpu.VMEM((ncol, MC * L, LANE), jnp.float32),
            pltpu.SemaphoreType.DMA((ncol + 1,)),
        ],
        compiler_params=pltpu.CompilerParams(
            dimension_semantics=("arbitrary", "arbitrary"),
            vmem_limit_bytes=110 * 1024 * 1024),
    )(x, w1, w2, g, w_f, w_g, w_o)
    return out.reshape(B, T2, U, w_o.shape[1])
```

```python
import math

import jax
import jax.numpy as jnp
import jax.experimental.pallas as pl
import jax.experimental.pallas.tpu as pltpu
from jax import lax

N = 32
TAPS = 16
L = N - TAPS + 1
NC = 3 * (N // 2 - 1) + 2
MC = 240
LANE = 128
JT = 400


def _neg(a):
    return None if a is None else (-a[0], a[1])


def _add(a, b):
    if a is None:
        return b
    if b is None:
        return a
    if a[0] == b[0]:
        return (a[0], a[1] + b[1])
    return (1, a[1] - b[1]) if a[0] > 0 else (1, b[1] - a[1])


def _sub(a, b):
    return _add(a, _neg(b))


def _mul(a, c):
    if a is None or abs(c) < 1e-12:
        return None
    if abs(abs(c) - 1.0) < 1e-12:
        return a if c > 0 else _neg(a)
    return (1, a[1] * (c * a[0]))


def _val(a):
    return a[1] if a[0] > 0 else -a[1]


def _twiddle(re, im, c, s):
    if re is not None and im is not None and abs(abs(c) - abs(s)) < 1e-12:
        sg = 1.0 if c * s > 0 else -1.0
        return (_mul(_sub(re, _mul(im, sg)), c), _mul(_add(im, _mul(re, sg)), c))
    return (_sub(_mul(re, c), _mul(im, s)), _add(_mul(re, s), _mul(im, c)))


def _rfft(x):
    n = len(x)
    if n == 1:
        return [(x[0], None)]
    if n == 2:
        return [(_add(x[0], x[1]), None), (_sub(x[0], x[1]), None)]
    e, o = _rfft(x[0::2]), _rfft(x[1::2])
    h, q = n // 2, n // 4
    out = [None] * (h + 1)
    out[0] = (_add(e[0][0], o[0][0]), None)
    out[h] = (_sub(e[0][0], o[0][0]), None)
    out[q] = (e[q][0], _neg(o[q][0]))
    for k in range(1, q):
        a = 2 * math.pi * k / n
        tr, ti = _twiddle(o[k][0], o[k][1], math.cos(a), -math.sin(a))
        out[k] = (_add(e[k][0], tr), _add(e[k][1], ti))
        out[h - k] = (_sub(e[k][0], tr), _sub(ti, e[k][1]))
    return out


def _irfft(X, need):
    h = len(X) - 1
    n = 2 * h
    if n == 2:
        return {i: (_add if i == 0 else _sub)(X[0][0], X[1][0]) for i in need}
    q = n // 4
    ne = sorted(i // 2 for i in need if i % 2 == 0)
    no = sorted(i // 2 for i in need if i % 2 == 1)
    out = {}
    if ne:
        e = [None] * (q + 1)
        e[0] = (_add(X[0][0], X[h][0]), None)
        e[q] = (X[q][0], None)
        for k in range(1, q):
            e[k] = (_add(X[k][0], X[h - k][0]), _sub(X[k][1], X[h - k][1]))
        out.update({2 * i: v for i, v in _irfft(e, ne).items()})
    if no:
        o = [None] * (q + 1)
        o[0] = (_sub(X[0][0], X[h][0]), None)
        o[q] = (_neg(X[q][1]), None)
        for k in range(1, q):
            a = 2 * math.pi * k / n
            o[k] = _twiddle(_sub(X[k][0], X[h - k][0]), _add(X[k][1], X[h - k][1]),
                            math.cos(a), math.sin(a))
        out.update({2 * i + 1: v for i, v in _irfft(o, no).items()})
    return out


def _data_components(x):
    X = _rfft(x)
    out = [X[0][0], X[N // 2][0]]
    for k in range(1, N // 2):
        out += [_add(X[k][0], X[k][1]), X[k][1], X[k][0]]
    return out


def _weight_components(w):
    W = _rfft(w)
    out = [W[0][0], W[N // 2][0]]
    for k in range(1, N // 2):
        vr, vi = _add(W[k][0], W[k][0]), _neg(_add(W[k][1], W[k][1]))
        out += [vr, _neg(_add(vr, vi)), _sub(vi, vr)]
    return out


def _gelu(x):
    c = math.sqrt(2.0 / math.pi)
    return (0.5 * x) * (1.0 + jnp.tanh(x * (c + (c * 0.044715) * (x * x))))


def _kernel(x_hbm, w1_hbm, w2_hbm, g_ref, wf_ref, wg_ref, wo_ref, out_ref,
            xs0, xs1, wraw, wh1, wh2, xh0, xh1, yh0, yh1, hs0, hs1, fb, fes, sems,
            *, T, K, D, U):
    b, s = pl.program_id(0), pl.program_id(1)
    T1 = T // 2
    NCOL = D // LANE
    f32, bf16 = jnp.float32, jnp.bfloat16
    xs, hs = (xs0, xs1), (hs0, hs1)
    NB = N // 2 - 1
    GPI = MC // 8 // NB

    def x_copy(bb, c):
        return pltpu.make_async_copy(x_hbm.at[bb, :, pl.ds(c * LANE, LANE)],
                                     xs[bb].bitcast(bf16).at[c, pl.ds(TAPS, T), :],
                                     sems.at[bb * NCOL + c])

    def weights(wh):
        def step(i):
            r = pl.multiple_of((i // NCOL) * 16, 16)
            c = pl.multiple_of((i % NCOL) * LANE, LANE)
            for ph in range(2):
                taps = []
                for m in range(N):
                    k = 2 * m - 1 + ph
                    ok = m < TAPS and 0 <= k < K
                    taps.append((1, wraw[k, pl.ds(r, 16), pl.ds(c, LANE)].astype(f32) * (1.0 / N))
                                if ok else None)
                for j, v in enumerate(_weight_components(taps)):
                    wh[j, pl.ds(ph * D + r, 16), pl.ds(c, LANE)] = _val(v).astype(bf16)
        return step
    NW = (D // 16) * NCOL

    def forward(load, xh):
        def step(i):
            r = pl.multiple_of(i * 8, 8)
            for c in range(NCOL):
                for ph, sig in enumerate(load(r, c)):
                    for j, v in enumerate(_data_components([(1, t) for t in sig])):
                        xh[j, pl.ds(r, 8), pl.ds(ph * D + c * LANE, LANE)] = _val(v).astype(bf16)
        return step

    def inverse(yh, emit):
        def step(i):
            r = pl.multiple_of(i * 8, 8)
            for c in range(NCOL):
                ld = lambda j: (1, yh[j, pl.ds(r, 8), pl.ds(c * LANE, LANE)])
                X = [(ld(0), None)] + [(ld(2 * k), ld(2 * k + 1)) for k in range(1, N // 2)]
                X.append((ld(1), None))
                y = _irfft(X, list(range(L)))
                for n in range(L):
                    emit(r, c, n, _gelu(_val(y[n])))
        return step

    def load_x(bb, b0):
        def load(r, c):
            w = [xs[bb][c, pl.ds((b0 + r) * L + m, 8, stride=L), :] for m in range(N)]
            yield [pltpu.bitcast(t << 16, f32) for t in w]
            yield [pltpu.bitcast(t & jnp.uint32(0xFFFF0000), f32) for t in w]
        return load

    def load_h(bb):
        def load(r, c):
            for ph in range(2):
                yield [hs[bb][c, pl.ds(r * 2 * L + 2 * m + ph, 8, stride=2 * L), :]
                       for m in range(N)]
        return load

    def emit_h(bb, b0):
        def emit(r, c, n, v):
            p0 = (b0 + r) * L + n
            hs[bb][c, pl.ds(TAPS + p0, 8, stride=L), :] = v
        return emit

    def emit_f(bb):
        def emit(r, c, n, v):
            fb[bb, n, pl.ds(r, 8), pl.ds(c * LANE, LANE)] = v.astype(bf16)
        return emit

    def zero_h_tail(bb):
        n = hs[bb].shape[1] - TAPS - T1
        for c in range(NCOL):
            hs[bb][c, pl.ds(TAPS + T1, n), :] = jnp.zeros((n, LANE), f32)

    def loop(lo, hi, *steps):
        def body(i, _):
            for st in steps:
                st(i)
        lax.fori_loop(lo, hi, body, None)

    def stage(xh, wh, yh, *side):
        dot = lambda j: jnp.dot(xh[j], wh[j], preferred_element_type=f32)
        yh[0] = dot(0)
        yh[1] = dot(1)

        def step(k):
            k1 = dot(3 * k + 2)
            yh[2 * k + 2] = k1 + dot(3 * k + 3)
            yh[2 * k + 3] = k1 + dot(3 * k + 4)
            for q in range(GPI):
                for st in side:
                    st(k * GPI + q)
        loop(0, NB, step)

    @pl.when(jnp.logical_and(b == 0, s == 0))
    def _():
        G8 = MC // 8
        cw1 = pltpu.make_async_copy(w1_hbm, wraw, sems.at[2 * NCOL])
        cw2 = pltpu.make_async_copy(w2_hbm, wraw, sems.at[2 * NCOL])
        cw1.start()
        for c in range(NCOL):
            x_copy(0, c).start()
        for bb in range(2):
            for c in range(NCOL):
                tail = xs0.shape[1] - TAPS // 2 - T1
                xs[bb][c, pl.ds(0, TAPS // 2), :] = jnp.zeros((TAPS // 2, LANE), jnp.uint32)
                xs[bb][c, pl.ds(TAPS // 2 + T1, tail), :] = jnp.zeros((tail, LANE), jnp.uint32)
                hs[bb][c, pl.ds(0, TAPS), :] = jnp.zeros((TAPS, LANE), f32)
        cw1.wait()
        loop(0, NW, weights(wh1))
        cw2.start()
        for c in range(NCOL):
            x_copy(1, c).start()
        for c in range(NCOL):
            x_copy(0, c).wait()
        loop(0, G8, forward(load_x(0, 0), xh0))
        cw2.wait()
        loop(G8, NW, weights(wh2))
        stage(xh0, wh1, yh0, forward(load_x(0, MC), xh1), weights(wh2))
        for c in range(NCOL):
            x_copy(1, c).wait()
        stage(xh1, wh1, yh1, forward(load_x(1, 0), xh0), inverse(yh0, emit_h(0, 0)))
        stage(xh0, wh1, yh0, forward(load_x(1, MC), xh1), inverse(yh1, emit_h(0, MC)))
        zero_h_tail(0)
        stage(xh1, wh1, yh1, forward(load_h(0), xh0), inverse(yh0, emit_h(1, 0)))
        fwd = forward(load_h(1), xh1)
        stage(xh0, wh2, yh0, inverse(yh1, emit_h(1, MC)))
        zero_h_tail(1)
        loop(0, G8, fwd)
        stage(xh1, wh2, yh1, inverse(yh0, emit_f(0)))
        loop(0, G8, inverse(yh1, emit_f(1)))

    @pl.when(s == 0)
    def _():
        def fe_step(n):
            fe = jnp.dot(fb[b, n], wf_ref[...], preferred_element_type=f32)
            for c in range(NCOL):
                fes[c, pl.ds(n, MC, stride=L), :] = fe[:, c * LANE:(c + 1) * LANE]
        with jax.named_scope("fe"):
            loop(0, L, fe_step)

    ge = jnp.dot(g_ref[0], wg_ref[...], preferred_element_type=f32)
    G = 40

    def joint(i, _):
        t0 = s * JT + i * G
        rows = []
        for t in range(G):
            fe = jnp.concatenate([fes[c, pl.ds(t0 + t, 1), :] for c in range(NCOL)], axis=1)
            rows.append(jnp.tanh(fe + ge))
        j = jnp.concatenate(rows, axis=0).astype(bf16)
        o = jnp.dot(j, wo_ref[...], preferred_element_type=f32)
        out_ref[0, pl.ds(pl.multiple_of(i * G * U, G * U), G * U), :] = o.astype(bf16)
    with jax.named_scope("joint"):
        lax.fori_loop(0, JT // G, joint, None)


@jax.jit
def pallas_standalone__seq2seq_rnn_t_joint__speech_kernel(x, w1, w2, g, w_f, w_g, w_o):
    B, T, D = x.shape
    K, U = w1.shape[0], g.shape[1]
    T2 = T // 4
    assert B == 2 and (D // 16) * (D // LANE) >= MC // 8
    assert K == 2 * TAPS - 1 and T % 4 == 0 and T2 % JT == 0 and U == 8
    assert 2 * MC * L >= T // 2 and MC * L >= T2
    ncol = D // LANE
    rows = lambda n: -(-(2 * ((n - 1) * L + N)) // 16) * 16
    full = lambda a: pl.BlockSpec(a.shape, lambda b, s: (0,) * a.ndim)
    hbm = pl.BlockSpec(memory_space=pl.ANY)
    kern = lambda *refs: _kernel(*refs, T=T, K=K, D=D, U=U)
    out = pl.pallas_call(
        kern,
        grid=(B, T2 // JT),
        in_specs=[hbm, hbm, hbm, pl.BlockSpec((1, U, D), lambda b, s: (b, 0, 0)),
                  full(w_f), full(w_g), full(w_o)],
        out_specs=pl.BlockSpec((1, JT * U, w_o.shape[1]), lambda b, s: (b, s, 0)),
        out_shape=jax.ShapeDtypeStruct((B, T2 * U, w_o.shape[1]), x.dtype),
        scratch_shapes=(
            [pltpu.VMEM((ncol, rows(2 * MC) // 2, LANE), jnp.uint32)] * 2
            + [pltpu.VMEM((K, D, D), jnp.bfloat16)]
            + [pltpu.VMEM((NC, 2 * D, D), jnp.bfloat16)] * 2
            + [pltpu.VMEM((NC, MC, 2 * D), jnp.bfloat16)] * 2
            + [pltpu.VMEM((N, MC, D), jnp.float32)] * 2
            + [pltpu.VMEM((ncol, max(rows(MC), TAPS + 2 * MC * L + 8), LANE), jnp.float32)] * 2
            + [pltpu.VMEM((B, L, MC, D), jnp.bfloat16),
               pltpu.VMEM((ncol, MC * L, LANE), jnp.float32),
               pltpu.SemaphoreType.DMA((2 * ncol + 1,))]),
        compiler_params=pltpu.CompilerParams(
            dimension_semantics=("arbitrary", "arbitrary"),
            vmem_limit_bytes=124 * 1024 * 1024),
    )(x, w1, w2, g, w_f, w_g, w_o)
    return out.reshape(B, T2, U, w_o.shape[1])
```

```python
import math

import jax
import jax.numpy as jnp
import jax.experimental.pallas as pl
import jax.experimental.pallas.tpu as pltpu
from jax import lax

N = 32
TAPS = 16
L = N - TAPS + 1
NC = 3 * (N // 2 - 1) + 2
MC = 240
LANE = 128
MS = 3
KS = 2
JT = 400


class _Interleave:
    def __init__(self):
        self.queue, self.gap, self.count = [], 0, 0

    def tick(self, n=1):
        self.count += n
        if self.queue and self.count >= self.gap:
            self.count = 0
            self.queue.pop(0)()


_IL = _Interleave()


def _neg(a):
    return None if a is None else (-a[0], a[1])


def _add(a, b):
    if a is None:
        return b
    if b is None:
        return a
    _IL.tick()
    if a[0] == b[0]:
        return (a[0], a[1] + b[1])
    return (1, a[1] - b[1]) if a[0] > 0 else (1, b[1] - a[1])


def _sub(a, b):
    return _add(a, _neg(b))


def _mul(a, c):
    if a is None or abs(c) < 1e-12:
        return None
    if abs(abs(c) - 1.0) < 1e-12:
        return a if c > 0 else _neg(a)
    _IL.tick()
    return (1, a[1] * (c * a[0]))


def _val(a):
    return a[1] if a[0] > 0 else -a[1]


def _twiddle(re, im, c, s):
    if re is not None and im is not None and abs(abs(c) - abs(s)) < 1e-12:
        sg = 1.0 if c * s > 0 else -1.0
        return (_mul(_sub(re, _mul(im, sg)), c), _mul(_add(im, _mul(re, sg)), c))
    return (_sub(_mul(re, c), _mul(im, s)), _add(_mul(re, s), _mul(im, c)))


def _rfft(x):
    n = len(x)
    if n == 1:
        return [(x[0], None)]
    if n == 2:
        return [(_add(x[0], x[1]), None), (_sub(x[0], x[1]), None)]
    e, o = _rfft(x[0::2]), _rfft(x[1::2])
    h, q = n // 2, n // 4
    out = [None] * (h + 1)
    out[0] = (_add(e[0][0], o[0][0]), None)
    out[h] = (_sub(e[0][0], o[0][0]), None)
    out[q] = (e[q][0], _neg(o[q][0]))
    for k in range(1, q):
        a = 2 * math.pi * k / n
        tr, ti = _twiddle(o[k][0], o[k][1], math.cos(a), -math.sin(a))
        out[k] = (_add(e[k][0], tr), _add(e[k][1], ti))
        out[h - k] = (_sub(e[k][0], tr), _sub(ti, e[k][1]))
    return out


def _irfft(X, need):
    h = len(X) - 1
    n = 2 * h
    if n == 2:
        return {i: (_add if i == 0 else _sub)(X[0][0], X[1][0]) for i in need}
    q = n // 4
    ne = sorted(i // 2 for i in need if i % 2 == 0)
    no = sorted(i // 2 for i in need if i % 2 == 1)
    out = {}
    if ne:
        e = [None] * (q + 1)
        e[0] = (_add(X[0][0], X[h][0]), None)
        e[q] = (X[q][0], None)
        for k in range(1, q):
            e[k] = (_add(X[k][0], X[h - k][0]), _sub(X[k][1], X[h - k][1]))
        out.update({2 * i: v for i, v in _irfft(e, ne).items()})
    if no:
        o = [None] * (q + 1)
        o[0] = (_sub(X[0][0], X[h][0]), None)
        o[q] = (_neg(X[q][1]), None)
        for k in range(1, q):
            a = 2 * math.pi * k / n
            o[k] = _twiddle(_sub(X[k][0], X[h - k][0]), _add(X[k][1], X[h - k][1]),
                            math.cos(a), math.sin(a))
        out.update({2 * i + 1: v for i, v in _irfft(o, no).items()})
    return out


def _data_components(x):
    X = _rfft(x)
    out = [X[0][0], X[N // 2][0]]
    for k in range(1, N // 2):
        out += [_add(X[k][0], X[k][1]), X[k][1], X[k][0]]
    return out


def _weight_components(w):
    W = _rfft(w)
    out = [W[0][0], W[N // 2][0]]
    for k in range(1, N // 2):
        vr, vi = _add(W[k][0], W[k][0]), _neg(_add(W[k][1], W[k][1]))
        out += [vr, _neg(_add(vr, vi)), _sub(vi, vr)]
    return out


def _gelu(x):
    c = math.sqrt(2.0 / math.pi)
    _IL.tick(8)
    return (0.5 * x) * (1.0 + jnp.tanh(x * (c + (c * 0.044715) * (x * x))))


def _kernel(x_hbm, w1_hbm, w2_hbm, g_ref, wf_ref, wg_ref, wo_ref, out_ref,
            xs0, xs1, wraw, wh1, wh2, xh0, xh1, yh0, yh1, hs0, hs1, fb, fes, sems,
            *, T, K, D, U):
    b, s = pl.program_id(0), pl.program_id(1)
    T1 = T // 2
    NCOL = D // LANE
    f32, bf16 = jnp.float32, jnp.bfloat16
    xs, hs = (xs0, xs1), (hs0, hs1)
    NB = N // 2 - 1
    GPI = MC // 8 // NB

    def x_copy(bb, c):
        return pltpu.make_async_copy(x_hbm.at[bb, :, pl.ds(c * LANE, LANE)],
                                     xs[bb].bitcast(bf16).at[c, pl.ds(TAPS, T), :],
                                     sems.at[bb * NCOL + c])

    def weights(wh):
        def step(i):
            r = pl.multiple_of((i // NCOL) * 16, 16)
            c = pl.multiple_of((i % NCOL) * LANE, LANE)
            for ph in range(2):
                taps = []
                for m in range(N):
                    k = 2 * m - 1 + ph
                    ok = m < TAPS and 0 <= k < K
                    taps.append((1, wraw[k, pl.ds(r, 16), pl.ds(c, LANE)].astype(f32) * (1.0 / N))
                                if ok else None)
                for j, v in enumerate(_weight_components(taps)):
                    wh[j, pl.ds(ph * D + r, 16), pl.ds(c, LANE)] = _val(v).astype(bf16)
                yield
        return step
    NW = (D // 16) * NCOL

    def forward(load, xh):
        def step(i):
            r = pl.multiple_of(i * 8, 8)
            for c in range(NCOL):
                for ph, sig in enumerate(load(r, c)):
                    for j, v in enumerate(_data_components([(1, t) for t in sig])):
                        xh[j, pl.ds(r, 8), pl.ds(ph * D + c * LANE, LANE)] = _val(v).astype(bf16)
                    yield
        return step

    def inverse(yh, emit):
        def step(i):
            r = pl.multiple_of(i * 8, 8)
            for c in range(NCOL):
                ld = lambda j: (1, yh[j, pl.ds(r, 8), pl.ds(c * LANE, LANE)])
                X = [(ld(0), None)] + [(ld(2 * k), ld(2 * k + 1)) for k in range(1, N // 2)]
                X.append((ld(1), None))
                y = _irfft(X, list(range(L)))
                for n in range(L):
                    emit(r, c, n, _gelu(_val(y[n])))
                yield
        return step

    def load_x(bb, b0):
        def load(r, c):
            w = [xs[bb][c, pl.ds((b0 + r) * L + m, 8, stride=L), :] for m in range(N)]
            yield [pltpu.bitcast(t << 16, f32) for t in w]
            yield [pltpu.bitcast(t & jnp.uint32(0xFFFF0000), f32) for t in w]
        return load

    def load_h(bb):
        def load(r, c):
            for ph in range(2):
                yield [hs[bb][c, pl.ds(r * 2 * L + 2 * m + ph, 8, stride=2 * L), :]
                       for m in range(N)]
        return load

    def emit_h(bb, b0):
        def emit(r, c, n, v):
            p0 = (b0 + r) * L + n
            hs[bb][c, pl.ds(TAPS + p0, 8, stride=L), :] = v
        return emit

    def emit_f(bb):
        def emit(r, c, n, v):
            fb[bb, n, pl.ds(r, 8), pl.ds(c * LANE, LANE)] = v.astype(bf16)
        return emit

    def zero_h_tail(bb):
        n = hs[bb].shape[1] - TAPS - T1
        for c in range(NCOL):
            hs[bb][c, pl.ds(TAPS + T1, n), :] = jnp.zeros((n, LANE), f32)

    def fe_step(n):
        fe = jnp.dot(fb[b, n], wf_ref[...], preferred_element_type=f32)
        for c in range(NCOL):
            fes[c, pl.ds(n, MC, stride=L), :] = fe[:, c * LANE:(c + 1) * LANE]

    def loop(lo, hi, *steps):
        def body(i, _):
            for st in steps:
                for _ in st(i) or ():
                    pass
        lax.fori_loop(lo, hi, body, None)

    def stage(xh, wh, yh, *side):
        dot = lambda j: jnp.dot(xh[j], wh[j], preferred_element_type=f32)
        yh[0] = dot(0)
        yh[1] = dot(1)

        def step(k):
            k1, acc = {}, {}

            def piece(m, i, h):
                def run():
                    ms = pl.ds(m * (MC // MS), MC // MS)
                    ks = pl.ds(h * (2 * D // KS), 2 * D // KS)
                    d = jnp.dot(xh[3 * k + 2 + i, ms, ks], wh[3 * k + 2 + i, ks, :],
                                preferred_element_type=f32)
                    prev = acc[m] if h else (k1[m] if i else None)
                    acc[m] = d if prev is None else prev + d
                    if h == KS - 1:
                        if i:
                            yh[2 * k + 1 + i, ms, :] = acc[m]
                        else:
                            k1[m] = acc[m]
                return run
            _IL.queue = [piece(m, i, h) for i in range(3) for h in range(KS) for m in range(MS)]
            ops = GPI * NCOL * (270 if len(side) == 1 else 740)
            _IL.gap, _IL.count = ops // len(_IL.queue), ops
            for q in range(GPI):
                for st in side:
                    for _ in st(k * GPI + q):
                        pass
            while _IL.queue:
                _IL.queue.pop(0)()
        loop(0, NB, step)

    @pl.when(jnp.logical_and(b == 0, s == 0))
    def _():
        G8 = MC // 8
        cw1 = pltpu.make_async_copy(w1_hbm, wraw, sems.at[2 * NCOL])
        cw2 = pltpu.make_async_copy(w2_hbm, wraw, sems.at[2 * NCOL])
        cw1.start()
        for c in range(NCOL):
            x_copy(0, c).start()
        for bb in range(2):
            for c in range(NCOL):
                tail = xs0.shape[1] - TAPS // 2 - T1
                xs[bb][c, pl.ds(0, TAPS // 2), :] = jnp.zeros((TAPS // 2, LANE), jnp.uint32)
                xs[bb][c, pl.ds(TAPS // 2 + T1, tail), :] = jnp.zeros((tail, LANE), jnp.uint32)
                hs[bb][c, pl.ds(0, TAPS), :] = jnp.zeros((TAPS, LANE), f32)
        cw1.wait()
        loop(0, NW, weights(wh1))
        cw2.start()
        for c in range(NCOL):
            x_copy(1, c).start()
        for c in range(NCOL):
            x_copy(0, c).wait()
        loop(0, G8, forward(load_x(0, 0), xh0))
        cw2.wait()
        loop(G8, NW, weights(wh2))
        stage(xh0, wh1, yh0, forward(load_x(0, MC), xh1), weights(wh2))
        for c in range(NCOL):
            x_copy(1, c).wait()
        stage(xh1, wh1, yh1, forward(load_x(1, 0), xh0), inverse(yh0, emit_h(0, 0)))
        stage(xh0, wh1, yh0, forward(load_x(1, MC), xh1), inverse(yh1, emit_h(0, MC)))
        zero_h_tail(0)
        stage(xh1, wh1, yh1, forward(load_h(0), xh0), inverse(yh0, emit_h(1, 0)))
        fwd = forward(load_h(1), xh1)
        stage(xh0, wh2, yh0, inverse(yh1, emit_h(1, MC)))
        zero_h_tail(1)
        loop(0, G8, fwd)
        stage(xh1, wh2, yh1, inverse(yh0, emit_f(0)))
        inv = inverse(yh1, emit_f(1))
        loop(0, NB, fe_step, lambda i: (u for q in range(GPI) for u in inv(i * GPI + q)))
        loop(NB, L, fe_step)

    @pl.when(jnp.logical_and(b > 0, s == 0))
    def _():
        loop(0, L, fe_step)

    ge = jnp.dot(g_ref[0], wg_ref[...], preferred_element_type=f32)
    G = 200

    def joint(i, _):
        t0 = s * JT + i * G
        rows = []
        for t in range(G):
            fe = jnp.concatenate([fes[c, pl.ds(t0 + t, 1), :] for c in range(NCOL)], axis=1)
            rows.append(jnp.tanh(fe + ge))
        j = jnp.concatenate(rows, axis=0).astype(bf16)
        o = jnp.dot(j, wo_ref[...], preferred_element_type=f32)
        out_ref[0, pl.ds(pl.multiple_of(i * G * U, G * U), G * U), :] = o.astype(bf16)
    with jax.named_scope("joint"):
        lax.fori_loop(0, JT // G, joint, None, unroll=True)


@jax.jit
def pallas_standalone__seq2seq_rnn_t_joint__speech_kernel(x, w1, w2, g, w_f, w_g, w_o):
    B, T, D = x.shape
    K, U = w1.shape[0], g.shape[1]
    T2 = T // 4
    assert B == 2 and (D // 16) * (D // LANE) >= MC // 8
    assert K == 2 * TAPS - 1 and T % 4 == 0 and T2 % JT == 0 and U == 8
    assert 2 * MC * L >= T // 2 and MC * L >= T2
    ncol = D // LANE
    rows = lambda n: -(-(2 * ((n - 1) * L + N)) // 16) * 16
    full = lambda a: pl.BlockSpec(a.shape, lambda b, s: (0,) * a.ndim)
    hbm = pl.BlockSpec(memory_space=pl.ANY)
    kern = lambda *refs: _kernel(*refs, T=T, K=K, D=D, U=U)
    out = pl.pallas_call(
        kern,
        grid=(B, T2 // JT),
        in_specs=[hbm, hbm, hbm, pl.BlockSpec((1, U, D), lambda b, s: (b, 0, 0)),
                  full(w_f), full(w_g), full(w_o)],
        out_specs=pl.BlockSpec((1, JT * U, w_o.shape[1]), lambda b, s: (b, s, 0)),
        out_shape=jax.ShapeDtypeStruct((B, T2 * U, w_o.shape[1]), x.dtype),
        scratch_shapes=(
            [pltpu.VMEM((ncol, rows(2 * MC) // 2, LANE), jnp.uint32)] * 2
            + [pltpu.VMEM((K, D, D), jnp.bfloat16)]
            + [pltpu.VMEM((NC, 2 * D, D), jnp.bfloat16)] * 2
            + [pltpu.VMEM((NC, MC, 2 * D), jnp.bfloat16)] * 2
            + [pltpu.VMEM((N, MC, D), jnp.float32)] * 2
            + [pltpu.VMEM((ncol, max(rows(MC), TAPS + 2 * MC * L + 8), LANE), jnp.float32)] * 2
            + [pltpu.VMEM((B, L, MC, D), jnp.bfloat16),
               pltpu.VMEM((ncol, MC * L, LANE), jnp.float32),
               pltpu.SemaphoreType.DMA((2 * ncol + 1,))]),
        compiler_params=pltpu.CompilerParams(
            dimension_semantics=("arbitrary", "arbitrary"),
            vmem_limit_bytes=124 * 1024 * 1024),
    )(x, w1, w2, g, w_f, w_g, w_o)
    return out.reshape(B, T2, U, w_o.shape[1])
```
